```python
import os as _os
_os.environ.setdefault("JAX_PLATFORMS", "cpu")
import jax
import jax.numpy as jnp

def _softmax(x, axis=-1):
    return jax.nn.softmax(x, axis=axis)
def _gelu(x):
    return jax.nn.gelu(x, approximate=True)
def _silu(x):
    return jax.nn.silu(x)
def _sigmoid(x):
    return jax.nn.sigmoid(x)
def _layernorm(x, axis=-1, eps=1e-5):
    m = jnp.mean(x, axis=axis, keepdims=True)
    v = jnp.var(x, axis=axis, keepdims=True)
    return (x - m) / jnp.sqrt(v + eps)
def _scatter_add(tgt, idx, src, axis=0):
    return tgt.at[idx].add(src)
def _segment_sum(src, seg, n):
    return jax.ops.segment_sum(src, seg, n)
class _Rng:
    def __init__(self, key):
        self._k = key
    def _next(self):
        self._k, sub = jax.random.split(self._k)
        return sub
    def normal(self, shape):
        return jax.random.normal(self._next(), shape, dtype=jnp.bfloat16)
    def randint(self, lo, hi, shape):
        return jax.random.randint(self._next(), shape, lo, hi, dtype=jnp.int32)
    def uniform(self, shape, lo=0.0, hi=1.0):
        return jax.random.uniform(self._next(), shape, jnp.bfloat16, lo, hi)
    def permutation(self, n):
        return jax.random.permutation(self._next(), n)


kernel_name = 'standalone__dcn_v2_cross__recsys'

def setup_inputs():
    _rng = _Rng(jax.random.key(int.from_bytes(__import__("os").urandom(4), "little")))
    _w = (lambda a: (lambda t: t.astype(jnp.bfloat16) if jnp.issubdtype(t.dtype, jnp.floating) else t)(jnp.asarray(a)))
    B, F, D, L = 4096, 26, 128, 6
    Din = min(F * D, 1024)
    return {
        "x0": _w((lambda *s: _rng.normal(s) * 0.05)(B, Din)),
        "ws": _w((lambda *s: _rng.normal(s) * 0.05)(L, Din, Din)),
        "bs": _w((lambda *s: _rng.normal(s) * 0.05)(L, Din)),
    }

def reference(x0, ws, bs):
    x = x0
    for l in range(ws.shape[0]):
        x = x0 * (x @ ws[l] + bs[l]) + x
    return x
```

```python
import jax
import jax.numpy as jnp
from jax import lax
import jax.experimental.pallas as pl
import jax.experimental.pallas.tpu as pltpu

_HEAD_ROWS = 256
_BLOCK_ROWS = 480


def _cross(x0, x, w, b):
    y = jnp.dot(x, w, preferred_element_type=jnp.float32)
    return (x0.astype(jnp.float32) * (y + b) + x.astype(jnp.float32)).astype(x.dtype)


def _kernel(x_hbm, w_hbm, b_hbm, o_hbm,
            xh, oh, xbuf, obuf, wbuf, bbuf, hsem, xsem, osem, wsem):
    B = x_hbm.shape[0]
    L = w_hbm.shape[0]
    h, bm = _HEAD_ROWS, _BLOCK_ROWS
    nb = (B - h) // bm

    def x_copy(i, s):
        return pltpu.make_async_copy(
            x_hbm.at[pl.ds(h + i * bm, bm)], xbuf.at[s], xsem.at[s])

    def o_copy(i, s):
        return pltpu.make_async_copy(
            obuf.at[s], o_hbm.at[pl.ds(h + i * bm, bm)], osem.at[s])

    def w_copy(l):
        return pltpu.make_async_copy(w_hbm.at[l], wbuf.at[l], wsem.at[l])

    b_copy = pltpu.make_async_copy(b_hbm, bbuf, hsem.at[0])
    xh_copy = pltpu.make_async_copy(x_hbm.at[pl.ds(0, h)], xh, hsem.at[1])
    oh_copy = pltpu.make_async_copy(oh, o_hbm.at[pl.ds(0, h)], hsem.at[2])

    xh_copy.start()
    w_copy(0).start()
    b_copy.start()
    xh_copy.wait()
    b_copy.wait()
    oh[...] = xh[...]
    bias = bbuf[...].astype(jnp.float32)

    def head(l, _):
        w_copy(l).wait()

        @pl.when(l == 0)
        def _():
            w_copy(1).start()

        @pl.when(l + 2 < L)
        def _():
            w_copy(l + 2).start()

        @pl.when(l + 1 == L)
        def _():
            x_copy(0, 0).start()

        row = lax.broadcasted_iota(jnp.int32, bias.shape, 0) == l
        b = jnp.sum(jnp.where(row, bias, 0.0), axis=0, keepdims=True)
        oh[...] = _cross(xh[...], oh[...], wbuf[l], b)

    lax.fori_loop(0, L, head, None)
    oh_copy.start()

    def body(i, _):
        s = i % 2

        @pl.when(i + 1 < nb)
        def _():
            x_copy(i + 1, 1 - s).start()

        x_copy(i, s).wait()

        @pl.when(i >= 2)
        def _():
            o_copy(i - 2, s).wait()

        x = xbuf[s]
        for l in range(L):
            x = _cross(xbuf[s], x, wbuf[l], bbuf[l:l + 1, :].astype(jnp.float32))
        obuf[s] = x
        o_copy(i, s).start()

    lax.fori_loop(0, nb, body, None)
    oh_copy.wait()
    for i in range(max(nb - 2, 0), nb):
        o_copy(i, i % 2).wait()


@jax.jit
def pallas_standalone__dcn_v2_cross__recsys_kernel(
    x0: jax.Array,
    ws: jax.Array,
    bs: jax.Array,
):
    B, D = x0.shape
    L = ws.shape[0]
    h, bm = _HEAD_ROWS, _BLOCK_ROWS
    assert L >= 2 and B > h and (B - h) % bm == 0
    hbm = pl.BlockSpec(memory_space=pl.ANY)
    return pl.pallas_call(
        _kernel,
        in_specs=[hbm, hbm, hbm],
        out_specs=hbm,
        out_shape=jax.ShapeDtypeStruct((B, D), x0.dtype),
        scratch_shapes=[
            pltpu.VMEM((h, D), x0.dtype),
            pltpu.VMEM((h, D), x0.dtype),
            pltpu.VMEM((2, bm, D), x0.dtype),
            pltpu.VMEM((2, bm, D), x0.dtype),
            pltpu.VMEM((L, D, D), ws.dtype),
            pltpu.VMEM((L, D), bs.dtype),
            pltpu.SemaphoreType.DMA((3,)),
            pltpu.SemaphoreType.DMA((2,)),
            pltpu.SemaphoreType.DMA((2,)),
            pltpu.SemaphoreType.DMA((L,)),
        ],
        compiler_params=pltpu.CompilerParams(
            vmem_limit_bytes=100 * 2**20, disable_bounds_checks=True),
    )(x0, ws, bs)
```
